```python
import os as _os
_os.environ.setdefault("JAX_PLATFORMS", "cpu")
import jax
import jax.numpy as jnp

def _softmax(x, axis=-1):
    return jax.nn.softmax(x, axis=axis)
def _gelu(x):
    return jax.nn.gelu(x, approximate=True)
def _silu(x):
    return jax.nn.silu(x)
def _sigmoid(x):
    return jax.nn.sigmoid(x)
def _layernorm(x, axis=-1, eps=1e-5):
    m = jnp.mean(x, axis=axis, keepdims=True)
    v = jnp.var(x, axis=axis, keepdims=True)
    return (x - m) / jnp.sqrt(v + eps)
def _scatter_add(tgt, idx, src, axis=0):
    return tgt.at[idx].add(src)
def _segment_sum(src, seg, n):
    return jax.ops.segment_sum(src, seg, n)
class _Rng:
    def __init__(self, key):
        self._k = key
    def _next(self):
        self._k, sub = jax.random.split(self._k)
        return sub
    def normal(self, shape):
        return jax.random.normal(self._next(), shape, dtype=jnp.bfloat16)
    def randint(self, lo, hi, shape):
        return jax.random.randint(self._next(), shape, lo, hi, dtype=jnp.int32)
    def uniform(self, shape, lo=0.0, hi=1.0):
        return jax.random.uniform(self._next(), shape, jnp.bfloat16, lo, hi)
    def permutation(self, n):
        return jax.random.permutation(self._next(), n)


kernel_name = 'gated_mix__linear_attn_block__sliding_local_dilated__prompt'

def setup_inputs():
    _rng = _Rng(jax.random.key(int.from_bytes(__import__("os").urandom(4), "little")))
    _w = (lambda a: (lambda t: t.astype(jnp.bfloat16) if jnp.issubdtype(t.dtype, jnp.floating) else t)(jnp.asarray(a)))
    def _A_setup():
        B, S, D = 1, 2048, 512
        return {
            "x": _w((lambda *s: _rng.normal(s) * 0.05)(B, S, D)),
            "wqkv": _w((lambda *s: _rng.normal(s) * 1.6)(D, 3 * D)),
            "wo": _w((lambda *s: _rng.normal(s) * 0.8)(D, D)),
        }
    _A_in = _A_setup()

    def _B_setup():
        B, S, D = 1, 2048, 512
        return {
            "x": _w((lambda *s: _rng.normal(s) * 0.05)(B, S, D)),
            "wqkv": _w((lambda *s: _rng.normal(s) * 0.8)(D, 3 * D)),
            "wo": _w((lambda *s: _rng.normal(s) * 0.05)(D, D)),
        }
    _B_in = _B_setup()

    return {
        "A_x": _A_in["x"],
        "A_wqkv": _A_in["wqkv"],
        "A_wo": _A_in["wo"],
        "B_x": _B_in["x"],
        "B_wqkv": _B_in["wqkv"],
        "B_wo": _B_in["wo"],
        "gate_w": _w((lambda *s: _rng.normal(s) * 0.05)(512) * 16.0),
    }

def reference(A_x, A_wqkv, A_wo, B_x, B_wqkv, B_wo, gate_w):
    def _A_ref(x, wqkv, wo):
        B, S, D = x.shape
        H = 32; Dh = D // H
        qkv = (lambda x, *d: x.transpose(*d))((x @ wqkv).reshape(B, S, 3, H, Dh), 2, 0, 3, 1, 4)
        q, k, v = qkv[0], qkv[1], qkv[2]
        phi = lambda t: jnp.where(t > 0, t + 1, jnp.exp(t)) + 1e-6
        pq, pk = phi(q), phi(k)
        kv = jnp.einsum("bhsd,bhse->bhde", pk, v)
        z = jnp.einsum("bhsd->bhd", pk)
        num = jnp.einsum("bhqd,bhde->bhqe", pq, kv)
        den = jnp.einsum("bhqd,bhd->bhq", pq, z)[..., None] + 1e-6
        o = num / den
        return (lambda x, *d: x.transpose(*d))(o, 0, 2, 1, 3).reshape(B, S, D) @ wo

    def _B_ref(x, wqkv, wo):
        B, S, D = x.shape
        H = 32; Dh = D // H
        W, dil = 8, 2
        qkv = (lambda x, *d: x.transpose(*d))((x @ wqkv).reshape(B, S, 3, H, Dh), 2, 0, 3, 1, 4)
        q, k, v = qkv[0], qkv[1], qkv[2]
        scale = Dh ** -0.5
        pos = jnp.arange(S)
        off = jnp.arange(W) * dil
        idx = pos[:, None] - off[None, :]
        mask = idx >= 0
        idx_c = jnp.where(mask, idx, 0).reshape(-1)
        kg = k[:, :, idx_c, :].reshape(B, H, S, W, Dh)
        vg = v[:, :, idx_c, :].reshape(B, H, S, W, Dh)
        logits = jnp.einsum("bhsd,bhswd->bhsw", q, kg) * scale
        logits = jnp.where(mask[None, None, :, :], logits, -1e9)
        attn = _softmax(logits, axis=-1)
        o = jnp.einsum("bhsw,bhswd->bhsd", attn, vg)
        return (lambda x, *d: x.transpose(*d))(o, 0, 2, 1, 3).reshape(B, S, D) @ wo

    x = A_x
    g = _sigmoid((x * gate_w).sum(-1, keepdims=True))
    a = _A_ref(x, A_wqkv, A_wo)
    b = _B_ref(x, B_wqkv, B_wo)
    return g * a + (1 - g) * b
```

```python
import functools
import jax
import jax.numpy as jnp
from jax import lax
import jax.experimental.pallas as pl
import jax.experimental.pallas.tpu as pltpu

S, D, H, DH, W, DIL = 2048, 512, 32, 16, 8, 2
BS = 256
NB = S // BS
HALO = 16
ANY = pl.BlockSpec(memory_space=pl.ANY)
SLAB = 16
FLAGS = {"XLA_TPU_EVENLY_DISTRIBUTE_CRITICAL_NODES": True}
F32, BF16 = jnp.float32, jnp.bfloat16
NT = (((1,), (1,)), ((), ()))


def _dot(a, b):
    return jnp.dot(a, b, preferred_element_type=F32)


def _phi(t):
    return jnp.where(t > 0, t + 1.0, jnp.exp(t)) + 1e-6


def _recip(x):
    r = pl.reciprocal(x, approx=True)
    return r * (2.0 - x * r)


def kernel(ax_ref, wk_ref, h0, h1, h2, h3, gw_ref, o_ref,
           wkt, g_acc, z_acc, m_s, zm_s, wb_s, wob_s, qs, ks, vs, tr, obs, awqkv_ref, awo_ref, bwqkv_ref, bwo_ref, sems, xs, wq):
    cps = [pltpu.make_async_copy(h, d, sems.at[n]) for n, (h, d) in enumerate(
        ((h2, bwqkv_ref), (h3, bwo_ref), (h0, awqkv_ref), (h1, awo_ref)))]
    p = pl.program_id(0)
    i = pl.program_id(1)

    @pl.when((p == 0) & (i == 0))
    def _():
        for cp in cps:
            cp.start()
        wkt[...] = wk_ref[...].astype(F32).T.astype(BF16)
        g_acc[...] = jnp.zeros_like(g_acc)
        z_acc[...] = jnp.zeros_like(z_acc)

    def phase0():
        x = ax_ref[...]
        xs[i] = x
        kt = lax.dot_general(wkt[...], x, NT, preferred_element_type=F32)
        pk = _phi(kt)
        zz = z_acc[...]
        for j in range(BS // 128):
            zz = zz + pk[:, j * 128:(j + 1) * 128]
        z_acc[...] = zz
        g_acc[...] += _dot(pk.astype(BF16), x)

    def perm(kc):
        sl = slice(kc * 128, (kc + 1) * 128)
        for t in range(3):
            wt = bwqkv_ref[sl, t * D:(t + 1) * D].astype(F32).T
            if t == 0:
                wt = wt * (DH ** -0.5)
            tr[t] = wt
        tr[3] = bwo_ref[:, sl].astype(F32)
        for t in range(4):
            for d in range(DH):
                r = tr[t, pl.ds(d, H, stride=DH), :].astype(BF16)
                if t < 3:
                    wb_s[t * D + d * H:t * D + (d + 1) * H, sl] = r
                else:
                    wob_s[d * H:(d + 1) * H, sl] = r

    pl.when((p == 0) & (i < NB - 4))(phase0)
    for kc in range(4):
        @pl.when((p == 0) & (i == NB - 4 + kc))
        def _(kc=kc):
            if kc == 0:
                cps[0].wait()
                cps[1].wait()
            phase0()
            perm(kc)

    def project(x, slot, t):
        r = lax.dot_general(x, wb_s[t * D:(t + 1) * D, :], NT, preferred_element_type=F32)
        for c in range(4):
            v = r[:, c * 128:(c + 1) * 128]
            if t == 0:
                qs[slot, c] = v
            else:
                (ks if t == 1 else vs)[slot, c, HALO:, :] = v
        return r

    def gate(x):
        return jax.nn.sigmoid(jnp.sum(x.astype(F32) * gw_ref[...].astype(F32).reshape(1, D), axis=-1, keepdims=True))

    def attn(cur, blk, g, s0):
        q = [qs[cur, c, s0:s0 + SLAB, :] for c in range(4)]
        ls = []
        for w in range(W):
            off = HALO + s0 - DIL * w
            t = q[0] * ks[cur, 0, off:off + SLAB, :]
            for c in range(1, 4):
                t = t + q[c] * ks[cur, c, off:off + SLAB, :]
            t = t + pltpu.roll(t, 64, 1)
            t = t + pltpu.roll(t, 32, 1)
            if blk == 0 and s0 < DIL * w:
                pos = lax.broadcasted_iota(jnp.int32, (SLAB, 128), 0) + (s0 - DIL * w)
                t = jnp.where(pos >= 0, t, -1e9)
            ls.append(t)
        m = functools.reduce(jnp.maximum, ls)
        es = [jnp.exp(l - m) for l in ls]
        ssum = functools.reduce(lambda a, b: a + b, es)
        sc = (1.0 - g[s0:s0 + SLAB]) * _recip(ssum)
        for c in range(4):
            acc = None
            for w in range(W):
                off = HALO + s0 - DIL * w
                t = es[w] * vs[cur, c, off:off + SLAB, :]
                acc = t if acc is None else acc + t
            obs[cur, s0:s0 + SLAB, c * 128:(c + 1) * 128] = (acc * sc).astype(BF16)

    nsl = BS // SLAB
    per = nsl // 4

    def halo(cur, nxt):
        for c in range(4):
            ks[nxt, c, 0:HALO, :] = ks[cur, c, BS:BS + HALO, :]
            vs[nxt, c, 0:HALO, :] = vs[cur, c, BS:BS + HALO, :]

    @pl.when((p == 1) & (i == 0))
    def _():
        cps[2].wait()
        cps[3].wait()
        r = lax.broadcasted_iota(jnp.int32, (128, 128), 0) // DH
        c = lax.broadcasted_iota(jnp.int32, (128, 128), 1) // DH
        same = r == c
        z = jnp.sum(z_acc[...], axis=1, keepdims=True)
        x = xs[0]
        wq[...] = awqkv_ref[:, 0:D]
        for t in (1, 2, 0):
            r = project(x, 0, t)
            if t > 0:
                for c in range(4):
                    (ks if t == 1 else vs)[0, c, 0:HALO, :] = jnp.broadcast_to(r[0:1, c * 128:(c + 1) * 128], (HALO, 128))
        halo(0, 1)
        g = gate(x)
        xn = xs[1]
        for t in range(4):
            if t < 3:
                project(xn, 1, t)
            else:
                for cc in range(4):
                    sl = slice(cc * 128, (cc + 1) * 128)
                    kv = _dot(g_acc[sl, :].astype(BF16), awqkv_ref[:, 2 * D + cc * 128:2 * D + (cc + 1) * 128])
                    kv = jnp.where(same, kv, 0.0).astype(BF16)
                    m_s[sl, :] = _dot(kv, awo_ref[sl, :]).astype(BF16)
                    zm_s[sl, :] = jnp.where(same, jnp.broadcast_to(z[sl], (128, 128)), 0.0).astype(BF16)
            for s in range(per * t, per * (t + 1)):
                attn(0, 0, g, s * SLAB)

    def main(do_proj, do_attn):
        cur = i % 2
        nxt = 1 - cur
        xa = xs[i]
        if do_attn:
            gn = gate(xs[i + 1])
        if do_proj:
            halo(nxt, cur)
            x2 = xs[i + 2]

        def pa():
            g = gate(xa)
            pq = _phi(_dot(xa, wq[...]))
            pqb = pq.astype(BF16)
            den = jnp.concatenate(
                [_dot(pqb[:, c * 128:(c + 1) * 128], zm_s[c * 128:(c + 1) * 128, :]) for c in range(4)], axis=1) + 1e-6
            oa = (pq * (g * _recip(den))).astype(BF16)
            return oa
        st = {}
        pieces = [lambda: st.update(oa=pa())]
        if do_proj:
            pieces += [functools.partial(project, x2, cur, t) for t in (1, 2, 0)]
        def fin():
            o_ref[...] = (_dot(st['oa'], m_s[...]) + _dot(obs[cur], wob_s[...])).astype(o_ref.dtype)
        pieces.append(fin)
        n = len(pieces)
        for j, f in enumerate(pieces):
            f()
            if do_attn:
                for s in range(nsl * j // n, nsl * (j + 1) // n):
                    attn(nxt, 1, gn, s * SLAB)

    pl.when((p == 1) & (i < NB - 2))(functools.partial(main, True, True))
    pl.when((p == 1) & (i == NB - 2))(functools.partial(main, False, True))
    pl.when((p == 1) & (i == NB - 1))(functools.partial(main, False, False))


@jax.jit
def pallas_gated_mix__linear_attn_block__sliding_local_dilated__prompt_kernel(
        A_x, A_wqkv, A_wo, B_x, B_wqkv, B_wo, gate_w):
    full = lambda shape: pl.BlockSpec(shape, lambda p, i: (0, 0))
    x2 = A_x.reshape(S, D)
    out = pl.pallas_call(
        kernel,
        grid=(2, NB),
        in_specs=[
            pl.BlockSpec((BS, D), lambda p, i: (jnp.maximum(i, p * (NB - 1)), 0)),
            pl.BlockSpec((D, D), lambda p, i: (0, 1)),
            ANY, ANY, ANY, ANY, pl.BlockSpec((D,), lambda p, i: (0,)),
        ],
        out_specs=pl.BlockSpec((BS, D), lambda p, i: (p * i, 0)),
        out_shape=jax.ShapeDtypeStruct((S, D), BF16),
        scratch_shapes=[
            pltpu.VMEM((D, D), BF16), pltpu.VMEM((D, D), F32), pltpu.VMEM((D, 128), F32),
            pltpu.VMEM((D, D), BF16), pltpu.VMEM((D, 128), BF16),
            pltpu.VMEM((3 * D, D), BF16), pltpu.VMEM((D, D), BF16),
            pltpu.VMEM((2, 4, BS, 128), F32),
            pltpu.VMEM((2, 4, HALO + BS, 128), F32), pltpu.VMEM((2, 4, HALO + BS, 128), F32),
            pltpu.VMEM((4, D, 128), F32), pltpu.VMEM((2, BS, D), BF16),
            pltpu.VMEM((D, 3 * D), BF16), pltpu.VMEM((D, D), BF16), pltpu.VMEM((D, 3 * D), BF16), pltpu.VMEM((D, D), BF16),
            pltpu.SemaphoreType.DMA((4,)), pltpu.VMEM((NB, BS, D), BF16), pltpu.VMEM((D, D), BF16),
        ],
        compiler_params=pltpu.CompilerParams(
            dimension_semantics=("arbitrary", "arbitrary"), vmem_limit_bytes=100 * 1024 * 1024, flags=FLAGS),
    )(x2, A_wqkv, A_wqkv, A_wo, B_wqkv, B_wo, gate_w)
    return out.reshape(1, S, D)
```

```python
import functools
import jax
import jax.numpy as jnp
from jax import lax
import jax.experimental.pallas as pl
import jax.experimental.pallas.tpu as pltpu

S, D, H, DH, W, DIL = 2048, 512, 32, 16, 8, 2
BS = 256
NB = S // BS
HALO = 16
ANY = pl.BlockSpec(memory_space=pl.ANY)
SLAB = 16
FLAGS = {"XLA_TPU_EVENLY_DISTRIBUTE_CRITICAL_NODES": True}
F32, BF16 = jnp.float32, jnp.bfloat16
NT = (((1,), (1,)), ((), ()))


def _dot(a, b):
    return jnp.dot(a, b, preferred_element_type=F32)


def _phi(t):
    return jnp.where(t > 0, t + 1.0, jnp.exp(t)) + 1e-6


def _recip(x):
    r = pl.reciprocal(x, approx=True)
    return r * (2.0 - x * r)


def kernel(ax_ref, wk_ref, h0, h1, h2, h3, gw_ref, o_ref,
           wkt, g_acc, z_acc, m_s, zm_s, wb_s, wob_s, qs, ks, vs, tr, obs, awqkv_ref, awo_ref, bwqkv_ref, bwo_ref, sems, xs, wq, gs, ps):
    cps = [pltpu.make_async_copy(h, d, sems.at[n]) for n, (h, d) in enumerate(
        ((h2, bwqkv_ref), (h3, bwo_ref), (h0, awqkv_ref), (h1, awo_ref)))]
    p = pl.program_id(0)
    i = pl.program_id(1)

    @pl.when((p == 0) & (i == 0))
    def _():
        for cp in cps:
            cp.start()
        wkt[...] = wk_ref[...].astype(F32).T.astype(BF16)
        g_acc[...] = jnp.zeros_like(g_acc)
        z_acc[...] = jnp.zeros_like(z_acc)

    def gate(x):
        return jax.nn.sigmoid(jnp.sum(x.astype(F32) * gw_ref[...].astype(F32).reshape(1, D), axis=-1, keepdims=True))

    def getx(j):
        return jnp.concatenate([xs[j, c] for c in range(4)], axis=1)

    def phase0():
        x = ax_ref[...]
        for c in range(4):
            xs[i, c] = x[:, c * 128:(c + 1) * 128]
        gs[i] = jnp.broadcast_to(gate(x), (BS, 128))
        kt = lax.dot_general(wkt[...], x, NT, preferred_element_type=F32)
        pk = _phi(kt)
        zz = z_acc[...]
        for j in range(BS // 128):
            zz = zz + pk[:, j * 128:(j + 1) * 128]
        z_acc[...] = zz
        g_acc[...] += _dot(pk.astype(BF16), x)

    def perm(kc):
        sl = slice(kc * 128, (kc + 1) * 128)
        for t in range(3):
            wt = bwqkv_ref[sl, t * D:(t + 1) * D].astype(F32).T
            if t == 0:
                wt = wt * (DH ** -0.5 * 1.4426950408889634)
            tr[t] = wt
        tr[3] = bwo_ref[:, sl].astype(F32)
        for t in range(4):
            for d in range(DH):
                r = tr[t, pl.ds(d, H, stride=DH), :].astype(BF16)
                if t < 3:
                    wb_s[t * D + d * H:t * D + (d + 1) * H, sl] = r
                else:
                    wob_s[d * H:(d + 1) * H, sl] = r

    pl.when((p == 0) & (i < NB - 4))(phase0)
    for kc in range(4):
        @pl.when((p == 0) & (i == NB - 4 + kc))
        def _(kc=kc):
            if kc == 0:
                cps[0].wait()
                cps[1].wait()
            phase0()
            perm(kc)

    def project(x, slot, t):
        r = lax.dot_general(x, wb_s[t * D:(t + 1) * D, :], NT, preferred_element_type=F32)
        for c in range(4):
            v = r[:, c * 128:(c + 1) * 128]
            if t == 0:
                qs[slot, c] = v
            else:
                (ks if t == 1 else vs)[slot, c, HALO:, :] = v
        return r

    def attn(cur, blk, s0, first=True):
        q = [qs[cur, c, s0:s0 + SLAB, :] for c in range(4)]
        ls = []
        for w in range(W):
            off = HALO + s0 - DIL * w
            t = q[0] * ks[cur, 0, off:off + SLAB, :]
            for c in range(1, 4):
                t = t + q[c] * ks[cur, c, off:off + SLAB, :]
            t = t + pltpu.roll(t, 64, 1)
            t = t + pltpu.roll(t, 32, 1)
            if first and s0 < DIL * w:
                pos = lax.broadcasted_iota(jnp.int32, (SLAB, 128), 0) + (s0 - DIL * w)
                t = jnp.where(pos >= 0, t, -1e9)
            ls.append(t)
        m = functools.reduce(jnp.maximum, ls)
        es = [jnp.exp2(l - m) for l in ls]
        ssum = functools.reduce(lambda a, b: a + b, es)
        sc = (1.0 - gs[blk, s0:s0 + SLAB, :]) * _recip(ssum)
        for w in range(W):
            ps[w, s0:s0 + SLAB, :] = es[w] * sc

    def pv(cur, s0):
        es = [ps[w, s0:s0 + SLAB, :] for w in range(W)]
        for c in range(4):
            acc = None
            for w in range(W):
                off = HALO + s0 - DIL * w
                t = es[w] * vs[cur, c, off:off + SLAB, :]
                acc = t if acc is None else acc + t
            obs[cur, s0:s0 + SLAB, c * 128:(c + 1) * 128] = acc.astype(BF16)

    nsl = BS // SLAB
    per = nsl // 4

    def halo(cur, nxt):
        for c in range(4):
            ks[nxt, c, 0:HALO, :] = ks[cur, c, BS:BS + HALO, :]
            vs[nxt, c, 0:HALO, :] = vs[cur, c, BS:BS + HALO, :]

    @pl.when((p == 1) & (i == 0))
    def _():
        cps[2].wait()
        cps[3].wait()
        r = lax.broadcasted_iota(jnp.int32, (128, 128), 0) // DH
        c = lax.broadcasted_iota(jnp.int32, (128, 128), 1) // DH
        same = r == c
        z = jnp.sum(z_acc[...], axis=1, keepdims=True)
        x = getx(0)
        wq[...] = awqkv_ref[:, 0:D]
        for t in (1, 2, 0):
            r = project(x, 0, t)
            if t > 0:
                for c in range(4):
                    (ks if t == 1 else vs)[0, c, 0:HALO, :] = jnp.broadcast_to(r[0:1, c * 128:(c + 1) * 128], (HALO, 128))
        halo(0, 1)
        xn = getx(1)
        for t in range(4):
            if t < 3:
                project(xn, 1, (2, 1, 0)[t])
            else:
                for cc in range(4):
                    sl = slice(cc * 128, (cc + 1) * 128)
                    kv = _dot(g_acc[sl, :].astype(BF16), awqkv_ref[:, 2 * D + cc * 128:2 * D + (cc + 1) * 128])
                    kv = jnp.where(same, kv, 0.0).astype(BF16)
                    m_s[sl, :] = _dot(kv, awo_ref[sl, :]).astype(BF16)
                    zm_s[sl, :] = jnp.where(same, jnp.broadcast_to(z[sl], (128, 128)), 0.0).astype(BF16)
            for s in range((0, 6, 11, 16, 16)[t], (6, 11, 16, 16)[t]):
                attn(0, 0, s * SLAB)
            for s in range((0, 0, 6, 11)[t], (0, 6, 11, 16)[t]):
                pv(0, s * SLAB)

    def main(do_proj, do_attn):
        cur = i % 2
        nxt = 1 - cur
        xa = getx(i)
        if do_proj:
            halo(nxt, cur)
            x2 = getx(i + 2)

        def pa():
            g = jnp.concatenate([gs[i]] * 4, axis=1)
            pq = _phi(_dot(xa, wq[...]))
            pqb = pq.astype(BF16)
            den = jnp.concatenate(
                [_dot(pqb[:, c * 128:(c + 1) * 128], zm_s[c * 128:(c + 1) * 128, :]) for c in range(4)], axis=1) + 1e-6
            oa = (pq * (g * _recip(den))).astype(BF16)
            return oa
        st = {}
        pieces = [lambda: st.update(oa=pa())]
        if do_proj:
            pieces += [functools.partial(project, x2, cur, t) for t in (1, 2, 0)]
        def fin():
            o_ref[...] = (_dot(st['oa'], m_s[...]) + _dot(obs[cur], wob_s[...])).astype(o_ref.dtype)
        pieces.append(fin)
        L = lambda lo, hi: [attn(nxt, i + 1, s * SLAB, False) for s in range(lo, hi)] if do_attn else None
        PV = lambda lo, hi: [pv(nxt, s * SLAB) for s in range(lo, hi)] if do_attn else None
        h = nsl // 2
        if do_proj:
            pa_, pk_, pv_, pq_, fin_ = pieces
            pv_(); L(0,6); pk_(); L(6,11); PV(0,6); pq_(); L(11,16); PV(6,11); pa_(); PV(11,16); fin_()
        else:
            L(0, nsl); pieces[0](); PV(0, nsl); pieces[1]()

    pl.when((p == 1) & (i < NB - 2))(functools.partial(main, True, True))
    pl.when((p == 1) & (i == NB - 2))(functools.partial(main, False, True))
    pl.when((p == 1) & (i == NB - 1))(functools.partial(main, False, False))


@jax.jit
def pallas_gated_mix__linear_attn_block__sliding_local_dilated__prompt_kernel(
        A_x, A_wqkv, A_wo, B_x, B_wqkv, B_wo, gate_w):
    full = lambda shape: pl.BlockSpec(shape, lambda p, i: (0, 0))
    x2 = A_x.reshape(S, D)
    out = pl.pallas_call(
        kernel,
        grid=(2, NB),
        in_specs=[
            pl.BlockSpec((BS, D), lambda p, i: (jnp.maximum(i, p * (NB - 1)), 0)),
            pl.BlockSpec((D, D), lambda p, i: (0, 1)),
            ANY, ANY, ANY, ANY, pl.BlockSpec((D,), lambda p, i: (0,)),
        ],
        out_specs=pl.BlockSpec((BS, D), lambda p, i: (p * i, 0)),
        out_shape=jax.ShapeDtypeStruct((S, D), BF16),
        scratch_shapes=[
            pltpu.VMEM((D, D), BF16), pltpu.VMEM((D, D), F32), pltpu.VMEM((D, 128), F32),
            pltpu.VMEM((D, D), BF16), pltpu.VMEM((D, 128), BF16),
            pltpu.VMEM((3 * D, D), BF16), pltpu.VMEM((D, D), BF16),
            pltpu.VMEM((2, 4, BS, 128), F32),
            pltpu.VMEM((2, 4, HALO + BS, 128), F32), pltpu.VMEM((2, 4, HALO + BS, 128), F32),
            pltpu.VMEM((4, D, 128), F32), pltpu.VMEM((2, BS, D), BF16),
            pltpu.VMEM((D, 3 * D), BF16), pltpu.VMEM((D, D), BF16), pltpu.VMEM((D, 3 * D), BF16), pltpu.VMEM((D, D), BF16),
            pltpu.SemaphoreType.DMA((4,)), pltpu.VMEM((NB, 4, BS, 128), BF16), pltpu.VMEM((D, D), BF16), pltpu.VMEM((NB, BS, 128), F32), pltpu.VMEM((W, BS, 128), F32),
        ],
        compiler_params=pltpu.CompilerParams(
            dimension_semantics=("arbitrary", "arbitrary"), vmem_limit_bytes=100 * 1024 * 1024, flags=FLAGS),
    )(x2, A_wqkv, A_wqkv, A_wo, B_wqkv, B_wo, gate_w)
    return out.reshape(1, S, D)
```

```python
import functools
import jax
import jax.numpy as jnp
from jax import lax
import jax.experimental.pallas as pl
import jax.experimental.pallas.tpu as pltpu

S, D, H, DH, W, DIL = 2048, 512, 32, 16, 8, 2
BS = 256
NB = S // BS
HALO = 16
ANY = pl.BlockSpec(memory_space=pl.ANY)
SLAB = 16
FLAGS = {"XLA_TPU_EVENLY_DISTRIBUTE_CRITICAL_NODES": True}
F32, BF16 = jnp.float32, jnp.bfloat16
NT = (((1,), (1,)), ((), ()))


def _dot(a, b):
    return jnp.dot(a, b, preferred_element_type=F32)


def _phi(t):
    return jnp.where(t > 0, t + 1.0, jnp.exp(t)) + 1e-6


def _recip(x):
    r = pl.reciprocal(x, approx=True)
    return r * (2.0 - x * r)


def kernel(ax_ref, wk_ref, h0, h1, h2, h3, gw_ref, o_ref,
           wkt, g_acc, z_acc, m_s, zm_s, wb_s, wob_s, qs, ks, vs, tr, obs, awqkv_ref, awo_ref, bwqkv_ref, bwo_ref, sems, xs, wq, gs, ps):
    cps = [pltpu.make_async_copy(h, d, sems.at[n]) for n, (h, d) in enumerate(
        ((h2, bwqkv_ref), (h3, bwo_ref), (h0, awqkv_ref), (h1, awo_ref)))]
    p = pl.program_id(0)
    i = pl.program_id(1)

    @pl.when((p == 0) & (i == 0))
    def _():
        for cp in cps:
            cp.start()
        wkt[...] = wk_ref[...].astype(F32).T.astype(BF16)
        g_acc[...] = jnp.zeros_like(g_acc)
        z_acc[...] = jnp.zeros_like(z_acc)

    def gate(x):
        return jax.nn.sigmoid(jnp.sum(x.astype(F32) * gw_ref[...].astype(F32).reshape(1, D), axis=-1, keepdims=True))

    def getx(j):
        return jnp.concatenate([xs[j, c] for c in range(4)], axis=1)

    def phase0():
        x = ax_ref[...]
        for c in range(4):
            xs[i, c] = x[:, c * 128:(c + 1) * 128]
        gs[i] = jnp.broadcast_to(gate(x), (BS, 128))
        kt = lax.dot_general(wkt[...], x, NT, preferred_element_type=F32)
        pk = _phi(kt)
        zz = z_acc[...]
        for j in range(BS // 128):
            zz = zz + pk[:, j * 128:(j + 1) * 128]
        z_acc[...] = zz
        g_acc[...] += _dot(pk.astype(BF16), x)

    def perm(kc):
        sl = slice(kc * 128, (kc + 1) * 128)
        for t in range(3):
            wt = bwqkv_ref[sl, t * D:(t + 1) * D].astype(F32).T
            if t == 0:
                wt = wt * (DH ** -0.5 * 1.4426950408889634)
            tr[t] = wt
        tr[3] = bwo_ref[:, sl].astype(F32)
        tr[4] = awqkv_ref[sl, 0:D].astype(F32).T
        for t in range(5):
            for d in range(DH):
                r = tr[t, pl.ds(d, H, stride=DH), :].astype(BF16)
                if t < 3:
                    wb_s[t * D + d * H:t * D + (d + 1) * H, sl] = r
                elif t == 4:
                    wq[d * H:(d + 1) * H, sl] = r
                else:
                    wob_s[d * H:(d + 1) * H, sl] = r

    pl.when((p == 0) & (i < NB - 4))(phase0)
    for kc in range(4):
        @pl.when((p == 0) & (i == NB - 4 + kc))
        def _(kc=kc):
            if kc == 0:
                cps[0].wait()
                cps[1].wait()
                cps[2].wait()
            phase0()
            perm(kc)

    def project(x, slot, t):
        r = lax.dot_general(x, wb_s[t * D:(t + 1) * D, :], NT, preferred_element_type=F32)
        for c in range(4):
            v = r[:, c * 128:(c + 1) * 128]
            if t == 0:
                qs[slot, c] = v
            else:
                (ks if t == 1 else vs)[slot, c, HALO:, :] = v
        return r

    def attn(cur, blk, s0, first=True):
        q = [qs[cur, c, s0:s0 + SLAB, :] for c in range(4)]
        ls = []
        for w in range(W):
            off = HALO + s0 - DIL * w
            t = q[0] * ks[cur, 0, off:off + SLAB, :]
            for c in range(1, 4):
                t = t + q[c] * ks[cur, c, off:off + SLAB, :]
            t = t + pltpu.roll(t, 64, 1)
            t = t + pltpu.roll(t, 32, 1)
            if first and s0 < DIL * w:
                pos = lax.broadcasted_iota(jnp.int32, (SLAB, 128), 0) + (s0 - DIL * w)
                t = jnp.where(pos >= 0, t, -1e9)
            ls.append(t)
        m = functools.reduce(jnp.maximum, ls)
        es = [jnp.exp2(l - m) for l in ls]
        ssum = functools.reduce(lambda a, b: a + b, es)
        sc = (1.0 - gs[blk, s0:s0 + SLAB, :]) * _recip(ssum)
        for w in range(W):
            ps[w, s0:s0 + SLAB, :] = es[w] * sc

    def pv(cur, s0):
        es = [ps[w, s0:s0 + SLAB, :] for w in range(W)]
        for c in range(4):
            acc = None
            for w in range(W):
                off = HALO + s0 - DIL * w
                t = es[w] * vs[cur, c, off:off + SLAB, :]
                acc = t if acc is None else acc + t
            obs[cur, s0:s0 + SLAB, c * 128:(c + 1) * 128] = acc.astype(BF16)

    nsl = BS // SLAB
    per = nsl // 4

    def halo(cur, nxt):
        for c in range(4):
            ks[nxt, c, 0:HALO, :] = ks[cur, c, BS:BS + HALO, :]
            vs[nxt, c, 0:HALO, :] = vs[cur, c, BS:BS + HALO, :]

    @pl.when((p == 1) & (i == 0))
    def _():
        cps[3].wait()
        r = lax.broadcasted_iota(jnp.int32, (128, 128), 0) // DH
        c = lax.broadcasted_iota(jnp.int32, (128, 128), 1) // DH
        same = r == c
        z = jnp.sum(z_acc[...], axis=1, keepdims=True)
        x = getx(0)
        for t in (0, 1, 2):
            r = project(x, 0, t)
            if t > 0:
                for c in range(4):
                    (ks if t == 1 else vs)[0, c, 0:HALO, :] = jnp.broadcast_to(r[0:1, c * 128:(c + 1) * 128], (HALO, 128))
        halo(0, 1)
        xn = getx(1)
        for t in range(4):
            if t != 1:
                project(xn, 1, (2, 0, 1, 0)[t])
            else:
                for cc in range(4):
                    sl = slice(cc * 128, (cc + 1) * 128)
                    kv = _dot(g_acc[sl, :].astype(BF16), awqkv_ref[:, 2 * D + cc * 128:2 * D + (cc + 1) * 128])
                    kv = jnp.where(same, kv, 0.0).astype(BF16)
                    mm = _dot(kv, awo_ref[sl, :])
                    for c2 in range(4):
                        tr[c2, sl, :] = mm[:, c2 * 128:(c2 + 1) * 128]
                tr[4] = jnp.broadcast_to(z, (D, 128))
                for c2 in range(4):
                    for d in range(DH):
                        m_s[d * H:(d + 1) * H, c2 * 128:(c2 + 1) * 128] = tr[c2, pl.ds(d, H, stride=DH), :].astype(BF16)
                    zp = jnp.concatenate([tr[4, pl.ds(c2 * 4 + d, H, stride=DH), :] for d in range(4)], axis=0)
                    zm_s[c2] = zp.T[0:8, :]
            for s in range((0, 6, 11, 16, 16)[t], (6, 11, 16, 16)[t]):
                attn(0, 0, s * SLAB)
            for s in range((0, 0, 6, 11)[t], (0, 6, 11, 16)[t]):
                pv(0, s * SLAB)

    def main(do_proj, do_attn):
        cur = i % 2
        nxt = 1 - cur
        xa = getx(i)
        if do_proj:
            halo(nxt, cur)
            x2 = getx(i + 2)

        def pa():
            pq = _phi(lax.dot_general(xa, wq[...], NT, preferred_element_type=F32))
            pc = [pq[:, c * 128:(c + 1) * 128] for c in range(4)]
            t = pc[0] * zm_s[0, 0:1, :]
            for c in range(1, 4):
                t = t + pc[c] * zm_s[c, 0:1, :]
            t = t + pltpu.roll(t, 64, 1)
            t = t + pltpu.roll(t, 32, 1)
            f = gs[i] * _recip(t + 1e-6)
            oa = jnp.concatenate([(x_ * f).astype(BF16) for x_ in pc], axis=1)
            return oa
        st = {}
        pieces = [lambda: st.update(oa=pa())]
        if do_proj:
            pieces += [functools.partial(project, x2, cur, t) for t in (1, 2, 0)]
        def fin():
            o_ref[...] = (_dot(st['oa'], m_s[...]) + _dot(obs[cur], wob_s[...])).astype(o_ref.dtype)
        pieces.append(fin)
        L = lambda lo, hi: [attn(nxt, i + 1, s * SLAB, False) for s in range(lo, hi)] if do_attn else None
        PV = lambda lo, hi: [pv(nxt, s * SLAB) for s in range(lo, hi)] if do_attn else None
        h = nsl // 2
        if do_proj:
            pa_, pk_, pv_, pq_, fin_ = pieces
            L(0,3); pv_(); PV(0,3); pq_(); pa_(); L(3,13); L(13,16); pk_(); PV(3,13); PV(13,16); fin_()
        else:
            L(0, nsl); pieces[0](); PV(0, nsl); pieces[1]()

    pl.when((p == 1) & (i < NB - 2))(functools.partial(main, True, True))
    pl.when((p == 1) & (i == NB - 2))(functools.partial(main, False, True))
    pl.when((p == 1) & (i == NB - 1))(functools.partial(main, False, False))


@jax.jit
def pallas_gated_mix__linear_attn_block__sliding_local_dilated__prompt_kernel(
        A_x, A_wqkv, A_wo, B_x, B_wqkv, B_wo, gate_w):
    full = lambda shape: pl.BlockSpec(shape, lambda p, i: (0, 0))
    x2 = A_x.reshape(S, D)
    out = pl.pallas_call(
        kernel,
        grid=(2, NB),
        in_specs=[
            pl.BlockSpec((BS, D), lambda p, i: (jnp.maximum(i, p * (NB - 1)), 0)),
            pl.BlockSpec((D, D), lambda p, i: (0, 1)),
            ANY, ANY, ANY, ANY, pl.BlockSpec((D,), lambda p, i: (0,)),
        ],
        out_specs=pl.BlockSpec((BS, D), lambda p, i: (p * i, 0)),
        out_shape=jax.ShapeDtypeStruct((S, D), BF16),
        scratch_shapes=[
            pltpu.VMEM((D, D), BF16), pltpu.VMEM((D, D), F32), pltpu.VMEM((D, 128), F32),
            pltpu.VMEM((D, D), BF16), pltpu.VMEM((4, 8, 128), F32),
            pltpu.VMEM((3 * D, D), BF16), pltpu.VMEM((D, D), BF16),
            pltpu.VMEM((2, 4, BS, 128), F32),
            pltpu.VMEM((2, 4, HALO + BS, 128), F32), pltpu.VMEM((2, 4, HALO + BS, 128), F32),
            pltpu.VMEM((5, D, 128), F32), pltpu.VMEM((2, BS, D), BF16),
            pltpu.VMEM((D, 3 * D), BF16), pltpu.VMEM((D, D), BF16), pltpu.VMEM((D, 3 * D), BF16), pltpu.VMEM((D, D), BF16),
            pltpu.SemaphoreType.DMA((4,)), pltpu.VMEM((NB, 4, BS, 128), BF16), pltpu.VMEM((D, D), BF16), pltpu.VMEM((NB, BS, 128), F32), pltpu.VMEM((W, BS, 128), F32),
        ],
        compiler_params=pltpu.CompilerParams(
            dimension_semantics=("arbitrary", "arbitrary"), vmem_limit_bytes=100 * 1024 * 1024, flags=FLAGS),
    )(x2, A_wqkv, A_wqkv, A_wo, B_wqkv, B_wo, gate_w)
    return out.reshape(1, S, D)
```
